```python
import os as _os
_os.environ.setdefault("JAX_PLATFORMS", "cpu")
import jax
import jax.numpy as jnp

def _softmax(x, axis=-1):
    return jax.nn.softmax(x, axis=axis)
def _gelu(x):
    return jax.nn.gelu(x, approximate=True)
def _silu(x):
    return jax.nn.silu(x)
def _sigmoid(x):
    return jax.nn.sigmoid(x)
def _layernorm(x, axis=-1, eps=1e-5):
    m = jnp.mean(x, axis=axis, keepdims=True)
    v = jnp.var(x, axis=axis, keepdims=True)
    return (x - m) / jnp.sqrt(v + eps)
def _scatter_add(tgt, idx, src, axis=0):
    return tgt.at[idx].add(src)
def _segment_sum(src, seg, n):
    return jax.ops.segment_sum(src, seg, n)
class _Rng:
    def __init__(self, key):
        self._k = key
    def _next(self):
        self._k, sub = jax.random.split(self._k)
        return sub
    def normal(self, shape):
        return jax.random.normal(self._next(), shape, dtype=jnp.bfloat16)
    def randint(self, lo, hi, shape):
        return jax.random.randint(self._next(), shape, lo, hi, dtype=jnp.int32)
    def uniform(self, shape, lo=0.0, hi=1.0):
        return jax.random.uniform(self._next(), shape, jnp.bfloat16, lo, hi)
    def permutation(self, n):
        return jax.random.permutation(self._next(), n)


kernel_name = 'gated_mix__compressed_kv_cla__ssm_conv_h3__prompt'

def setup_inputs():
    _rng = _Rng(jax.random.key(int.from_bytes(__import__("os").urandom(4), "little")))
    _w = (lambda a: (lambda t: t.astype(jnp.bfloat16) if jnp.issubdtype(t.dtype, jnp.floating) else t)(jnp.asarray(a)))
    def _A_setup():
        B, H, Sq, Sk, D, M = 1, 32, 2048, 2048, 128, 1024
        Dc = 4 * D
        return {
            "x": _w((lambda *s: _rng.normal(s) * 0.05)(B, Sq, M)),
            "c_kv": _w((lambda *s: _rng.normal(s) * 0.8)(B, Sk, Dc)),
            "w_q": _w((lambda *s: _rng.normal(s) * 3.2)(M, H, D) * (M ** -0.5)),
            "w_uk": _w((lambda *s: _rng.normal(s) * 3.2)(Dc, H, D) * (Dc ** -0.5)),
            "w_uv": _w((lambda *s: _rng.normal(s) * 0.8)(Dc, H, D) * (Dc ** -0.5)),
            "w_o": _w((lambda *s: _rng.normal(s) * 0.8)(H, D, M) * ((H * D) ** -0.5)),
        }
    _A_in = _A_setup()

    def _B_setup():
        B, S, D = 1, 2048, 1024
        ks = 4
        return {
            "q": _w((lambda *s: _rng.normal(s) * 0.05)(B, S, D)),
            "k": _w((lambda *s: _rng.normal(s) * 0.8)(B, S, D)),
            "v": _w((lambda *s: _rng.normal(s) * 0.8)(B, S, D)),
            "shift_k": _w((lambda *s: _rng.normal(s) * 0.8)(D, ks) * 0.5),
            "ssm_k": _w((lambda *s: _rng.normal(s) * 0.8)(D, S) * (1.0 / S ** 0.5)),
            "ssm_D": _w((lambda *s: _rng.normal(s) * 0.8)(D)),
        }
    _B_in = _B_setup()

    return {
        "A_x": _A_in["x"],
        "A_c_kv": _A_in["c_kv"],
        "A_w_q": _A_in["w_q"],
        "A_w_uk": _A_in["w_uk"],
        "A_w_uv": _A_in["w_uv"],
        "A_w_o": _A_in["w_o"],
        "B_q": _B_in["q"],
        "B_k": _B_in["k"],
        "B_v": _B_in["v"],
        "B_shift_k": _B_in["shift_k"],
        "B_ssm_k": _B_in["ssm_k"],
        "B_ssm_D": _B_in["ssm_D"],
        "gate_w": _w((lambda *s: _rng.normal(s) * 0.05)(1024) * 16.0),
    }

def reference(A_x, A_c_kv, A_w_q, A_w_uk, A_w_uv, A_w_o, B_q, B_k, B_v, B_shift_k, B_ssm_k, B_ssm_D, gate_w):
    def _A_ref(x, c_kv, w_q, w_uk, w_uv, w_o):
        B, Sq, M = x.shape[0], x.shape[1], x.shape[2]
        Sk = c_kv.shape[1]
        H, D = w_q.shape[1], w_q.shape[2]
        q = jnp.einsum("bqm,mhd->bhqd", x, w_q)
        k = jnp.einsum("bkc,chd->bhkd", c_kv, w_uk)
        v = jnp.einsum("bkc,chd->bhkd", c_kv, w_uv)
        scores = jnp.einsum("bhqd,bhkd->bhqk", q, k) * (D ** -0.5)
        off = Sk - Sq
        qi = jnp.arange(Sq)[:, None]
        kj = jnp.arange(Sk)[None, :]
        cmask = kj <= (qi + off)
        scores = jnp.where(cmask[None, None], scores, -1e9)
        p = _softmax(scores, axis=-1)
        ctx = jnp.einsum("bhqk,bhkd->bhqd", p, v)
        return jnp.einsum("bhqd,hdm->bqm", ctx, w_o)

    def _B_ref(q, k, v, shift_k, ssm_k, ssm_D):
        B, S, D = q.shape
        ks = shift_k.shape[-1]
        k_pad = jnp.pad(k, ((0, 0), (ks - 1, 0), (0, 0)))
        k_shift = jnp.zeros_like(k)
        for t in range(ks):
            k_shift = k_shift + k_pad[:, t:t + S, :] * shift_k[:, ks - 1 - t][None, None, :]
        kv = k_shift * v
        L = 2 * S
        kv_pad = jnp.pad(kv, ((0, 0), (0, S), (0, 0)))
        kf_pad = jnp.pad(ssm_k, ((0, 0), (0, S)))
        kv_f = (lambda x, axes=(-2,-1): jnp.fft.rfft2(x.astype(jnp.float32), axes=axes))(kv_pad[:, None, :, :], axes=(1, 2))
        kf_f = (lambda x, axes=(-2,-1): jnp.fft.rfft2(x.astype(jnp.float32), axes=axes))(kf_pad[:, None, :], axes=(1, 2))
        kf_f = (lambda x, *d: x.transpose(*d))(kf_f, 1, 2, 0)
        y_f = kv_f * kf_f[None, :, :, :]
        y = (lambda x, s, axes=(-2,-1): jnp.fft.irfft2(x, s=s, axes=axes).astype(jnp.bfloat16))(y_f, (1, L), axes=(1, 2))[:, 0, :S, :]
        y = y + kv * ssm_D[None, None, :]
        return q * y

    x = A_x
    g = _sigmoid((x * gate_w).sum(-1, keepdims=True))
    a = _A_ref(x, A_c_kv, A_w_q, A_w_uk, A_w_uv, A_w_o)
    b = _B_ref(x, B_k, B_v, B_shift_k, B_ssm_k, B_ssm_D)
    return g * a + (1 - g) * b
```

```python
import functools
import os

import jax
import jax.numpy as jnp
import numpy as np
import jax.experimental.pallas as pl
import jax.experimental.pallas.tpu as pltpu

f32 = jnp.float32
bf16 = jnp.bfloat16
u32 = jnp.uint32

S = 2048
M = 1024
H = 32
D = 128
DC = 512
T = 128
NB = S // T
HP = 2
NSTEP = H // HP
HF = T // 2
KS = 4
LOG2E = 1.4426950408889634
NT = (((1,), (1,)), ((), ()))
NXC = 4
NU = int(os.environ.get("NU", "4"))
NEND = int(os.environ.get("NEND", "0"))
QAHEAD = int(os.environ.get("QAHEAD", "2"))
OLAG = int(os.environ.get("OLAG", "1"))
NTAIL = int(os.environ.get("NTAIL", "0"))


_MAC_ORDER = [15, 0, 14, 1, 13, 2, 12, 3, 11, 4, 10, 5, 9, 6, 8, 7]


def _pk(v):
    return pltpu.bitcast(v, u32)


def _upk(v):
    return pltpu.bitcast(v, bf16)


def _hs(a, b):
    return slice(a // 2, b // 2)


def _dft_tables():
    n = np.arange(T)[None, :]
    fw, inv = [], []
    for half in range(2):
        f = (np.arange(HF) * 2 + half)[:, None]
        th = 2.0 * np.pi * (f + 0.5) * n / (2 * T)
        m = np.concatenate([np.cos(th), -np.sin(th)], axis=0)
        fw.append(m)
        inv.append(m.T / T)
    return np.concatenate([np.stack(fw), np.stack(inv)], axis=0).astype(np.float32)


def _kernel(x_hbm, c_hbm, wq_hbm, wk_hbm, wv_hbm, wo_hbm, bk_hbm, bv_hbm, sh_hbm, hk_hbm,
            d_hbm, gw_hbm, tab_hbm, o_hbm,
            acc_ref, x_s, c_s, rq_s, rk_s, rv_s, wo_s, bk_s, bv_s, hk_s, sh_s, dr_s, gw_s, tab_s,
            wq_s, wkv_s, k_s, v_s, g_s, kp_s, d_s, o_s, z_s, kvd_s, u_s, ab_s, zm_s,
            sem_a, sem_kv, sem_x, sem_c, sem_small, sem_o):
    x32 = x_hbm.bitcast(u32)
    c32 = c_hbm.bitcast(u32)
    wq32 = wq_hbm.bitcast(u32)
    wk32 = wk_hbm.bitcast(u32)
    wv32 = wv_hbm.bitcast(u32)
    wo32 = wo_hbm.bitcast(u32)
    hk32 = hk_hbm.bitcast(u32)
    XR = S // 2 // NXC

    def a_copies(s):
        grp = s // 2
        if isinstance(s, int):
            cols = pl.ds(grp * T, T)
            hrow = pl.ds(grp * (T // 2), T // 2)
            orow = pl.ds(s * D, D)
        else:
            cols = pl.ds(pl.multiple_of(grp * T, T), T)
            hrow = pl.ds(pl.multiple_of(grp * (T // 2), T // 2), T // 2)
            orow = pl.ds(pl.multiple_of(s * D, D), D)
        return [
            pltpu.make_async_copy(hk32.at[hrow, :], hk_s, sem_a.at[0]),
            pltpu.make_async_copy(bk_hbm.at[:, cols], bk_s, sem_a.at[1]),
            pltpu.make_async_copy(bv_hbm.at[:, cols], bv_s, sem_a.at[2]),
            pltpu.make_async_copy(wq32.at[:, s, :], rq_s, sem_a.at[3]),
            pltpu.make_async_copy(wo32.at[orow, :], wo_s.at[s % 2], sem_a.at[4]),
        ]

    def kv_copies(s):
        return [
            pltpu.make_async_copy(wk32.at[:, s, :], rk_s, sem_kv.at[0]),
            pltpu.make_async_copy(wv32.at[:, s, :], rv_s, sem_kv.at[1]),
        ]

    def x_copy(j):
        return pltpu.make_async_copy(x32.at[pl.ds(j * XR, XR), :], x_s.at[pl.ds(j * XR, XR), :], sem_x.at[j])

    c_copy = pltpu.make_async_copy(c32, c_s, sem_c)

    small = [
        pltpu.make_async_copy(tab_hbm, tab_s, sem_small.at[0]),
        pltpu.make_async_copy(sh_hbm, sh_s, sem_small.at[1]),
        pltpu.make_async_copy(d_hbm, dr_s, sem_small.at[2]),
        pltpu.make_async_copy(gw_hbm, gw_s, sem_small.at[3]),
    ]

    def o_copy(i):
        r = pl.ds(i * T, T)
        return pltpu.make_async_copy(o_s.at[r, :], o_hbm.at[r, :], sem_o)

    scale = (D ** -0.5) * LOG2E

    def unpack_pair(w):
        lo = pltpu.bitcast(w << 16, f32)
        hi = pltpu.bitcast(w & jnp.uint32(0xFFFF0000), f32)
        return jnp.concatenate([lo, hi], axis=1).astype(bf16)

    def unpack_kv():
        wkv_s[:, :HP * D] = _pk(unpack_pair(rk_s[...]))
        wkv_s[:, HP * D:] = _pk(unpack_pair(rv_s[...]))

    def projkv(i):
        r = _hs(i * T, (i + 1) * T)
        kv = jnp.dot(_upk(c_s[r, :]), _upk(wkv_s[...]), preferred_element_type=f32)
        k_s[r, :] = _pk(kv[:, :HP * D].astype(bf16))
        v_s[r, :] = _pk(kv[:, HP * D:].astype(bf16))

    tail_blocks = list(range(NB - NTAIL, NB))

    def phase_a(s):
        slot = s % 2
        grp = s // 2
        for cp in a_copies(s): cp.wait()
        sgn = (1 - 2 * slot).astype(f32)
        cols = pl.ds(pl.multiple_of(grp * T, T), T)
        cv = dict(H={})
        ab = {}
        zmask = zm_s[...]

        def projkv_q(i, nq, deps):
            r0 = i * T // 2
            ntile = (T // 16) * (DC // T)
            rows = []
            deps = list(deps)
            assert len(deps) <= ntile
            pos = {(k * ntile) // len(deps): d for k, d in enumerate(deps)} if deps else {}
            for rg in range(T // 16):
                tiles = []
                for kt in range(DC // T):
                    tl = c_s[r0 + rg * 8:r0 + (rg + 1) * 8, kt * T:(kt + 1) * T]
                    idx = rg * (DC // T) + kt
                    if idx in pos:
                        tl = tl | (pltpu.bitcast(pos[idx], u32) & zmask)
                    tiles.append(tl)
                rows.append(jnp.concatenate(tiles, axis=1))
            lhs = jnp.concatenate(rows, axis=0)
            r = _hs(i * T, (i + 1) * T)
            kv = jnp.dot(_upk(lhs), _upk(wkv_s[:, nq * T:(nq + 1) * T]), preferred_element_type=f32)
            dst = k_s if nq < 2 else v_s
            dst[r, (nq % 2) * T:(nq % 2 + 1) * T] = _pk(kv.astype(bf16))

        def conv_h(m):
            hm = jax.lax.dot_general(tab_s[slot], _upk(hk_s[:, m * T:(m + 1) * T]), NT, preferred_element_type=f32)
            cv["H"][m] = hm
            hr, hi = hm[:HF], hm[HF:]
            if m > 0:
                hp = cv["H"][m - 1]
                hr = hr - sgn * hp[HF:]
                hi = hi + sgn * hp[:HF]
            ab[(0, m)] = hr
            ab[(1, m)] = hr + hi
            ab[(2, m)] = hi - hr

        def conv_prep(c):
            taps = cv["taps"]
            deps = []
            for q in range(T // 16):
                r0 = 8 + c * T + q * 16
                ks = kp_s[r0:r0 + 16, :] * taps[0:1, :]
                for j in range(1, KS):
                    ks = ks + kp_s[r0 - j:r0 - j + 16, :] * taps[j:j + 1, :]
                kv = ks * bv_s[r0 - 8:r0 + 8, :].astype(f32)
                kvd_s[r0 - 8:r0 + 8, :] = kv * cv["dvec"]
                u_s[r0 - 8:r0 + 8, :] = kv.astype(bf16)
                deps.append(kv[0:8] + kv[8:16])
            return deps

        def conv_u(c):
            u = jnp.dot(tab_s[slot], u_s[c * T:(c + 1) * T, :], preferred_element_type=f32)
            ur, ui = u[:HF], u[HF:]
            ab[(3, c)] = ur + ui
            ab[(4, c)] = ui
            ab[(5, c)] = ur

        def conv_mac(a, p0):
            ks = []
            for ty in range(3):
                t = ab[(ty, a)][p0:p0 + 8, :] * ab[(3 + ty, 0)][p0:p0 + 8, :]
                for c in range(1, a + 1):
                    t = t + ab[(ty, a - c)][p0:p0 + 8, :] * ab[(3 + ty, c)][p0:p0 + 8, :]
                ks.append(t)
            zr = ks[0] - ks[1]
            zi = ks[0] + ks[2]
            z_s[a * T + p0:a * T + p0 + 8, :] = zr
            z_s[a * T + HF + p0:a * T + HF + p0 + 8, :] = zi
            return [zr, zi]

        cv["taps"] = sh_s[:, cols].astype(f32)
        cv["dvec"] = d_s[pl.ds(grp, 1), :]
        kp_s[8:, :] = bk_s[...].astype(f32)
        for m in range(NB):
            conv_h(m)
        blocks = [i for i in range(NB) if i not in tail_blocks]
        quarters = [(i, nq) for i in blocks for nq in range(4)]
        G1 = int(os.environ.get("G1", "2"))
        G2 = int(os.environ.get("G2", "4"))
        pieces = [(a, p0) for p0 in range(0, HF, 8) for a in _MAC_ORDER]
        q0 = NB + G1 + G2
        nmb = len(quarters) - q0 - NEND
        tot = sum(a + 1 for a, _ in pieces)
        groups = [[] for _ in range(nmb)]
        accw = 0
        for (a, p0) in pieces:
            gi = min(nmb - 1, (accw * nmb) // tot)
            groups[gi].append((a, p0))
            accw += a + 1
        for k, (i, nq) in enumerate(quarters):
            deps = []
            if k < NB:
                deps = conv_prep(k)
            elif q0 <= k < q0 + nmb:
                for (a, p0) in groups[k - q0]:
                    deps += conv_mac(a, p0)
            projkv_q(i, nq, deps)
            if k == NB + G1 - 1:
                for c in range(NB):
                    conv_u(c)
        wq_s[...] = _pk(unpack_pair(rq_s[...]))

    def phase_b(s):
        slot = s % 2
        grp = s // 2
        cols = pl.ds(pl.multiple_of(grp * T, T), T)

        @pl.when(s + 1 < NSTEP)
        def _():
            for cp in kv_copies(s + 1): cp.wait()
            for cp in a_copies(s + 1): cp.start()

        row = jax.lax.broadcasted_iota(jnp.int32, (T, T), 0)
        col = jax.lax.broadcasted_iota(jnp.int32, (T, T), 1)
        tri = col <= row
        qv = {}

        def projq(i):
            r = _hs(i * T, (i + 1) * T)
            qv[i] = jnp.dot(_upk(x_s[r, :]), _upk(wq_s[...]), preferred_element_type=f32) * scale

        def scores(i, hh):
            cs = slice(hh * D, (hh + 1) * D)
            q = qv[i][:, cs].astype(bf16)
            return jax.lax.dot_general(q, _upk(k_s[_hs(0, (i + 1) * T), cs]), NT, preferred_element_type=f32)

        def softmax(i, sc):
            base = i * T
            dg = jnp.where(tri, sc[:, base:], -1e30)
            srow = jnp.concatenate([sc[:, :base], dg], axis=1) if base > 0 else dg
            m = jnp.max(srow, axis=-1, keepdims=True)
            p = jnp.exp2(srow - m)
            l = jnp.sum(p, axis=-1, keepdims=True)
            r = pl.reciprocal(l, approx=True)
            r = r * (2.0 - l * r)
            return p, g_s[base:base + T, :] * r

        def pv(i, hh, p, sc):
            cs = slice(hh * D, (hh + 1) * D)
            return jnp.dot(p.astype(bf16), _upk(v_s[_hs(0, (i + 1) * T), cs]), preferred_element_type=f32) * sc

        def conv_inv(a):
            r = slice(a * T, (a + 1) * T)
            y = jnp.dot(tab_s[2 + slot], z_s[r, :].astype(bf16), preferred_element_type=f32) + kvd_s[r, :]
            xc = _upk(x_s[_hs(a * T, (a + 1) * T), cols]).astype(f32)
            acc_ref[r, cols] += y * xc * (1.0 - g_s[r, :])

        def outp(i, ctxs):
            r = slice(i * T, (i + 1) * T)
            ctx = jnp.concatenate(ctxs, axis=1).astype(bf16)
            res = acc_ref[r, :] + jnp.dot(ctx, _upk(wo_s[slot]), preferred_element_type=f32)
            acc_ref[r, :] = res
            o_s[r, :] = res.astype(bf16)

            @pl.when(s == NSTEP - 1)
            def _():
                o_copy(i).start()

        order = list(range(NB - 1, -1, -1))
        for k in range(QAHEAD):
            projq(order[k])
        unpack_kv()

        @pl.when(s + 2 < NSTEP)
        def _():
            for cp in kv_copies(s + 2): cp.start()

        done = []
        tail = list(tail_blocks)
        for idx, i in enumerate(order):
            ss = [scores(i, hh) for hh in range(HP)]
            conv_inv(i)
            fill = []
            if idx + QAHEAD < NB:
                fill.append(functools.partial(projq, order[idx + QAHEAD]))
            if len(done) >= OLAG:
                fill.append(functools.partial(outp, *done.pop(0)))
            if NB - idx <= len(tail):
                fill.append(functools.partial(projkv, tail.pop(0)))
            ctxs = []
            for hh in range(HP):
                p, sc = softmax(i, ss[hh])
                if fill:
                    fill.pop(0)()
                ctxs.append(pv(i, hh, p, sc))
            for fn in fill:
                fn()
            done.append((i, ctxs))
        for d in done:
            outp(*d)

    for cp in kv_copies(0): cp.start()
    for cp in small: cp.start()
    c_copy.start()
    for cp in a_copies(0): cp.start()
    for j in range(NXC): x_copy(j).start()

    def zero_body(i, carry):
        acc_ref[pl.ds(pl.multiple_of(i * T, T), T), :] = jnp.zeros((T, M), f32)
        return carry
    jax.lax.fori_loop(0, NB, zero_body, 0)
    kp_s[0:8, :] = jnp.zeros((8, T), f32)
    zm_s[...] = jnp.zeros((8, T), u32)
    for cp in kv_copies(0): cp.wait()
    unpack_kv()
    for cp in kv_copies(1): cp.start()
    for cp in small: cp.wait()
    d_s[...] = dr_s[...].astype(f32) * 0.5
    c_copy.wait()
    for i in tail_blocks:
        projkv(i)

    def gate_body(i, carry):
        gw = gw_s[...].astype(f32)
        xf = _upk(x_s[pl.ds(pl.multiple_of(i * (T // 2), T // 2), T // 2), :]).astype(f32)
        t = xf[:, 0:T] * gw[0:1, :]
        for j in range(1, M // T):
            t = t + xf[:, j * T:(j + 1) * T] * gw[j:j + 1, :]
        z = jnp.sum(t, axis=-1, keepdims=True)
        g = 0.5 * jnp.tanh(0.5 * z) + 0.5
        g_s[pl.ds(pl.multiple_of(i * T, T), T), :] = jnp.broadcast_to(g, (T, T))
        return carry

    def loop_body(s, carry):
        @pl.when(s >= 0)
        def _():
            phase_b(s)

        @pl.when(s + 1 < NSTEP)
        def _():
            phase_a(s + 1)

        @pl.when(s < 0)
        def _():
            for j in range(NXC): x_copy(j).wait()
            jax.lax.fori_loop(0, NB, gate_body, 0, unroll=4)
        return carry

    jax.lax.fori_loop(-1, NSTEP, loop_body, 0)
    for i in range(NB):
        o_copy(i).wait()


@jax.jit
def pallas_gated_mix__compressed_kv_cla__ssm_conv_h3__prompt_kernel(
    A_x, A_c_kv, A_w_q, A_w_uk, A_w_uv, A_w_o, B_q, B_k, B_v, B_shift_k, B_ssm_k, B_ssm_D, gate_w,
):
    del B_q
    tab = _dft_tables()
    out = pl.pallas_call(
        _kernel,
        in_specs=[pl.BlockSpec(memory_space=pl.ANY)] * 13,
        out_specs=pl.BlockSpec(memory_space=pl.ANY),
        out_shape=jax.ShapeDtypeStruct((S, M), bf16),
        scratch_shapes=[
            pltpu.VMEM((S, M), f32),
            pltpu.VMEM((S // 2, M), u32),
            pltpu.VMEM((S // 2, DC), u32),
            pltpu.VMEM((M, D), u32),
            pltpu.VMEM((DC, D), u32),
            pltpu.VMEM((DC, D), u32),
            pltpu.VMEM((2, HP * D // 2, M), u32),
            pltpu.VMEM((S, T), bf16),
            pltpu.VMEM((S, T), bf16),
            pltpu.VMEM((T // 2, S), u32),
            pltpu.VMEM((KS, M), bf16),
            pltpu.VMEM((M // T, T), bf16),
            pltpu.VMEM((M // T, T), bf16),
            pltpu.VMEM((4, T, T), bf16),
            pltpu.VMEM((M // 2, HP * D), u32),
            pltpu.VMEM((DC // 2, 2 * HP * D), u32),
            pltpu.VMEM((S // 2, HP * D), u32),
            pltpu.VMEM((S // 2, HP * D), u32),
            pltpu.VMEM((S, T), f32),
            pltpu.VMEM((S + 8, T), f32),
            pltpu.VMEM((M // T, T), f32),
            pltpu.VMEM((S, M), bf16),
            pltpu.VMEM((S, T), f32),
            pltpu.VMEM((S, T), f32),
            pltpu.VMEM((S, T), bf16),
            pltpu.VMEM((6, NB, HF, T), f32),
            pltpu.VMEM((8, T), u32),
            pltpu.SemaphoreType.DMA((5,)),
            pltpu.SemaphoreType.DMA((2,)),
            pltpu.SemaphoreType.DMA((NXC,)),
            pltpu.SemaphoreType.DMA(()),
            pltpu.SemaphoreType.DMA((4,)),
            pltpu.SemaphoreType.DMA(()),
        ],
        compiler_params=pltpu.CompilerParams(
            vmem_limit_bytes=100 * 1024 * 1024,
            disable_bounds_checks=True,
        ),
    )(
        A_x.reshape(S, M), A_c_kv.reshape(S, DC), A_w_q, A_w_uk, A_w_uv, A_w_o.reshape(H * D, M),
        B_k.reshape(S, M), B_v.reshape(S, M), B_shift_k.T, B_ssm_k,
        B_ssm_D.reshape(M // T, T), gate_w.reshape(M // T, T),
        jnp.asarray(tab, bf16),
    )
    return out.reshape(1, S, M)
```

```python
import functools

import jax
import jax.numpy as jnp
import numpy as np
import jax.experimental.pallas as pl
import jax.experimental.pallas.tpu as pltpu

f32 = jnp.float32
bf16 = jnp.bfloat16
u32 = jnp.uint32

S = 2048
M = 1024
H = 32
D = 128
DC = 512
T = 128
NB = S // T
HP = 2
NSTEP = H // HP
HF = T // 2
KS = 4
LOG2E = 1.4426950408889634
NT = (((1,), (1,)), ((), ()))

QAHEAD = 2
OLAG = 2
UB0, NUB = 12, 4
G1, G2 = 2, 2
NUNP = 4
LAG = 4


def _pk(v):
    return pltpu.bitcast(v, u32)


def _upk(v):
    return pltpu.bitcast(v, bf16)


def _hs(a, b):
    return slice(a // 2, b // 2)


def _lo(w):
    return pltpu.bitcast(w << 16, f32)


def _hi(w):
    return pltpu.bitcast(w & jnp.uint32(0xFFFF0000), f32)


def _dft_tables():
    n = np.arange(T)[None, :]
    fw, inv = [], []
    for half in range(2):
        f = (np.arange(HF) * 2 + half)[:, None]
        th = 2.0 * np.pi * (f + 0.5) * n / (2 * T)
        m = np.concatenate([np.cos(th), -np.sin(th)], axis=0)
        fw.append(m)
        inv.append(m.T / T)
    perm = np.concatenate([np.arange(0, T, 2), np.arange(1, T, 2)])
    fwp = [m[:, perm] for m in fw]
    return np.concatenate([np.stack(fw), np.stack(inv), np.stack(fwp)], axis=0).astype(np.float32)


def _kernel(x_hbm, c_hbm, wq_hbm, wk_hbm, wv_hbm, wo_hbm, bk_hbm, bv_hbm, sh_hbm, hk_hbm,
            d_hbm, gw_hbm, tab_hbm, o_hbm,
            acc_ref, x_s, c_s, rq_s, rk_s, rv_s, wo_s, bk_s, bv_s, hk_s, sh_s, dr_s, gw_s, tab_s,
            wq_s, wkv_s, k_s, v_s, g_s, d_s, o_s, z_s, u_s, zm_s,
            sem_a, sem_kv, sem_xc, sem_small, sem_o):
    x32 = x_hbm.bitcast(u32)
    c32 = c_hbm.bitcast(u32)
    wq32 = wq_hbm.bitcast(u32)
    wk32 = wk_hbm.bitcast(u32)
    wv32 = wv_hbm.bitcast(u32)
    bk32 = bk_hbm.bitcast(u32)
    bv32 = bv_hbm.bitcast(u32)

    def blk(idx, size):
        if isinstance(idx, int):
            return pl.ds(idx * size, size)
        return pl.ds(pl.multiple_of(idx * size, size), size)

    def conv_copies(grp):
        return [
            pltpu.make_async_copy(hk_hbm.at[blk(grp, T), :], hk_s, sem_a.at[0]),
            pltpu.make_async_copy(bk32.at[:, blk(grp, T)], bk_s.at[pl.ds(8, S // 2), :], sem_a.at[1]),
            pltpu.make_async_copy(bv32.at[:, blk(grp, T)], bv_s, sem_a.at[2]),
        ]

    def q_copy(s):
        return pltpu.make_async_copy(wq32.at[:, s, :], rq_s, sem_a.at[3])

    def wo_copy(s):
        return pltpu.make_async_copy(wo_hbm.at[blk(s, HP * D), :], wo_s.at[s & 1], sem_a.at[4])

    def kv_copies(s):
        return [
            pltpu.make_async_copy(wk32.at[:, s, :], rk_s, sem_kv.at[0]),
            pltpu.make_async_copy(wv32.at[:, s, :], rv_s, sem_kv.at[1]),
        ]

    x_copy = pltpu.make_async_copy(x32, x_s, sem_xc.at[0])
    c_copy = pltpu.make_async_copy(c32, c_s, sem_xc.at[1])
    small = [
        pltpu.make_async_copy(tab_hbm, tab_s, sem_small.at[0]),
        pltpu.make_async_copy(sh_hbm, sh_s, sem_small.at[1]),
        pltpu.make_async_copy(d_hbm, dr_s, sem_small.at[2]),
        pltpu.make_async_copy(gw_hbm, gw_s, sem_small.at[3]),
    ]

    def o_copy(i):
        r = pl.ds(i * T, T)
        return pltpu.make_async_copy(o_s.at[r, :], o_hbm.at[r, :], sem_o)

    scale = (D ** -0.5) * LOG2E

    def unpack_pair(w):
        return jnp.concatenate([_lo(w), _hi(w)], axis=1).astype(bf16)

    def lhs_deps(ref, i, ncol, deps, zmask):
        r0 = i * T // 2
        if not deps:
            return ref[r0:r0 + T // 2, :]
        ntile = (T // 16) * (ncol // T)
        assert len(deps) <= ntile
        pos = {(k * ntile) // len(deps): d for k, d in enumerate(deps)}
        rows = []
        for rg in range(T // 16):
            tiles = []
            for kt in range(ncol // T):
                tl = ref[r0 + rg * 8:r0 + (rg + 1) * 8, kt * T:(kt + 1) * T]
                idx = rg * (ncol // T) + kt
                if idx in pos:
                    tl = tl | (pltpu.bitcast(pos[idx], u32) & zmask)
                tiles.append(tl)
            rows.append(jnp.concatenate(tiles, axis=1))
        return jnp.concatenate(rows, axis=0)

    def unpack_piece(src_ref, dst_ref, c0, r0):
        w = _pk(unpack_pair(src_ref[r0:r0 + 32, :]))
        dst_ref[r0 // 2:r0 // 2 + 16, c0:c0 + HP * D] = w
        return [w[0:8, 0:T] | w[8:16, 0:T] | w[0:8, T:] | w[8:16, T:]]

    def phase_a(s):
        slot = s & 1
        grp = s >> 1

        @pl.when(slot == 0)
        def _():
            for cp in conv_copies(grp):
                cp.wait()
        q_copy(s).wait()

        sgn = (1 - 2 * slot).astype(f32)
        zmask = zm_s[...]
        taps = sh_s[:, blk(grp, T)].astype(f32)
        dvec = d_s[pl.ds(grp, 1), :]
        hs = {}
        ab = {}
        k1 = {}

        def projkv_q(i, nq, deps):
            lhs = lhs_deps(c_s, i, DC, deps, zmask)
            r = _hs(i * T, (i + 1) * T)
            kv = jnp.dot(_upk(lhs), _upk(wkv_s[:, nq * T:(nq + 1) * T]), preferred_element_type=f32)
            dst = k_s if nq < 2 else v_s
            dst[r, (nq % 2) * T:(nq % 2 + 1) * T] = _pk(kv.astype(bf16))
            return pltpu.bitcast(kv[0:8, :], u32) & zmask

        def conv_h(m):
            hm = jax.lax.dot_general(tab_s[slot], hk_s[:, m * T:(m + 1) * T], NT,
                                     preferred_element_type=f32)
            hr, hi = hm[:HF], hm[HF:]
            if m == 0:
                hr = hr + dvec
            hs[m] = (hr, hi)
            if m > 0:
                pr, pi = hs[m - 1]
                hr = hr - sgn * pi
                hi = hi + sgn * pr
            ab[(0, m)] = hr
            ab[(1, m)] = hr + hi
            ab[(2, m)] = hi - hr

        def conv_prep(c):
            t0, t1, t2, t3 = [taps[j:j + 1, :] for j in range(KS)]
            deps = []
            for q in range(T // 32):
                r0 = c * HF + q * 16
                w0 = bk_s[8 + r0:8 + r0 + 16, :]
                w1 = bk_s[7 + r0:7 + r0 + 16, :]
                w2 = bk_s[6 + r0:6 + r0 + 16, :]
                e0, o0, e1, o1, o2 = _lo(w0), _hi(w0), _lo(w1), _hi(w1), _hi(w2)
                wv = bv_s[r0:r0 + 16, :]
                kve = (e0 * t0 + o1 * t1 + e1 * t2 + o2 * t3) * _lo(wv)
                kvo = (o0 * t0 + e0 * t1 + o1 * t2 + e1 * t3) * _hi(wv)
                u_s[c * T + q * 16:c * T + (q + 1) * 16, :] = kve.astype(bf16)
                u_s[c * T + HF + q * 16:c * T + HF + (q + 1) * 16, :] = kvo.astype(bf16)
                deps.append(kve[0:8] + kvo[0:8])
                deps.append(kve[8:16] + kvo[8:16])
            return deps

        def conv_u(c):
            u = jnp.dot(tab_s[4 + slot], u_s[c * T:(c + 1) * T, :], preferred_element_type=f32)
            ab[(4, c)] = u[HF:]
            ab[(5, c)] = u[:HF]

        def gated(v, tok):
            return pltpu.bitcast(pltpu.bitcast(v, u32) | tok, f32)

        def conv_mac(ty, p0, tok):
            sl = slice(p0, p0 + 8)
            a_ = [ab[(ty, m)][sl] for m in range(NB)]
            if ty == 0:
                b_ = [gated(ab[(5, c)][sl], tok) + ab[(4, c)][sl] for c in range(NB)]
            else:
                b_ = [gated(ab[(3 + ty, c)][sl], tok) for c in range(NB)]
            deps = []
            for a in range(NB):
                t = a_[a] * b_[0]
                for c in range(1, a + 1):
                    t = t + a_[a - c] * b_[c]
                if ty == 0:
                    k1[(a, p0)] = t
                elif ty == 1:
                    t = k1[(a, p0)] - t
                    z_s[a * T + p0:a * T + p0 + 8, :] = t
                else:
                    t = k1[(a, p0)] + t
                    z_s[a * T + HF + p0:a * T + HF + p0 + 8, :] = t
                deps.append(t)
            return deps

        quarters = [(i, nq) for i in range(NB) for nq in range(4)]
        projkv_q(*quarters.pop(0), [])
        for m in range(NB):
            conv_h(m)
        chunks = [(ty, p0) for p0 in range(0, HF, 8) for ty in range(3)]
        q0 = NB + G1 + G2
        nmb = len(quarters) - q0 - NUNP
        start = [q0 - 1 + (j * (nmb - LAG)) // len(chunks) for j in range(len(chunks))]
        pend = {}
        for k, (i, nq) in enumerate(quarters):
            deps = pend.pop(k, [])
            if k < NB:
                deps = conv_prep(k)
            elif k >= q0 + nmb:
                kk = k - q0 - nmb
                for r0 in range(kk * M // NUNP, (kk + 1) * M // NUNP, 32):
                    deps += unpack_piece(rq_s, wq_s, 0, r0)
            tok = projkv_q(i, nq, deps)
            for j, st in enumerate(start):
                if st == k:
                    pend.setdefault(k + LAG + 1, []).extend(conv_mac(*chunks[j], tok))
            if k == NB + G1 - 1:
                for c in range(NB):
                    conv_u(c)
        assert not pend

    def phase_b(s):
        slot = s & 1
        grp = s >> 1
        cols = blk(grp, T)

        wo_copy(s).wait()

        @pl.when(s + 1 < NSTEP)
        def _():
            q_copy(s + 1).start()
            wo_copy(s + 1).start()

        @pl.when(jnp.logical_and(s + 1 < NSTEP, slot == 1))
        def _():
            for cp in conv_copies(grp + 1):
                cp.start()

        @pl.when(s + 1 < NSTEP)
        def _():
            for cp in kv_copies(s + 1):
                cp.wait()

        row = jax.lax.broadcasted_iota(jnp.int32, (T, T), 0)
        col = jax.lax.broadcasted_iota(jnp.int32, (T, T), 1)
        tri = col <= row
        zmask = zm_s[...]
        qv = {}

        def projq(i):
            deps = []
            kk = UB0 - i
            if 0 <= kk < NUB:
                for r0 in range(kk * DC // NUB, (kk + 1) * DC // NUB, 32):
                    deps += unpack_piece(rk_s, wkv_s, 0, r0)
                    deps += unpack_piece(rv_s, wkv_s, HP * D, r0)
            lhs = lhs_deps(x_s, i, M, deps, zmask)
            qv[i] = jnp.dot(_upk(lhs), _upk(wq_s[...]), preferred_element_type=f32) * scale
            if kk == NUB - 1:
                @pl.when(s + 2 < NSTEP)
                def _():
                    for cp in kv_copies(s + 2):
                        cp.start()

        def scores(i, hh):
            cs = slice(hh * D, (hh + 1) * D)
            q = qv[i][:, cs].astype(bf16)
            return jax.lax.dot_general(q, _upk(k_s[_hs(0, (i + 1) * T), cs]), NT,
                                       preferred_element_type=f32)

        def softmax(i, sc):
            base = i * T
            dg = jnp.where(tri, sc[:, base:], -1e30)
            srow = jnp.concatenate([sc[:, :base], dg], axis=1) if base > 0 else dg
            m = jnp.max(srow, axis=-1, keepdims=True)
            p = jnp.exp2(srow - m)
            l = jnp.sum(p, axis=-1, keepdims=True)
            r = pl.reciprocal(l, approx=True)
            r = r * (2.0 - l * r)
            return p, g_s[base:base + T, :] * r

        def pv(i, hh, p, sc):
            cs = slice(hh * D, (hh + 1) * D)
            return jnp.dot(p.astype(bf16), _upk(v_s[_hs(0, (i + 1) * T), cs]),
                           preferred_element_type=f32) * sc

        def conv_inv(a):
            r = slice(a * T, (a + 1) * T)
            y = jnp.dot(tab_s[2 + slot], z_s[r, :].astype(bf16), preferred_element_type=f32)
            xc = _upk(x_s[_hs(a * T, (a + 1) * T), cols]).astype(f32)
            acc_ref[r, cols] += y * xc * (1.0 - g_s[r, :])

        def outp(i, ctxs):
            r = slice(i * T, (i + 1) * T)
            ctx = jnp.concatenate(ctxs, axis=1).astype(bf16)
            res = acc_ref[r, :] + jnp.dot(ctx, wo_s[slot], preferred_element_type=f32)
            acc_ref[r, :] = res
            o_s[r, :] = res.astype(bf16)

            @pl.when(s == NSTEP - 1)
            def _():
                o_copy(i).start()

        order = list(range(NB - 1, -1, -1))
        for k in range(QAHEAD):
            projq(order[k])
        done = []
        for idx, i in enumerate(order):
            ss = [scores(i, hh) for hh in range(HP)]
            fill = []
            if idx + QAHEAD < NB:
                fill.append(functools.partial(projq, order[idx + QAHEAD]))
            if len(done) >= OLAG:
                fill.append(functools.partial(outp, *done.pop(0)))
            ctxs = []
            for hh in range(HP):
                p, sc = softmax(i, ss[hh])
                if fill:
                    fill.pop(0)()
                ctxs.append(pv(i, hh, p, sc))
            conv_inv(i)
            for fn in fill:
                fn()
            done.append((i, ctxs))
        for d in done:
            outp(*d)

    for cp in kv_copies(0):
        cp.start()
    for cp in small:
        cp.start()
    c_copy.start()
    for cp in conv_copies(0):
        cp.start()
    q_copy(0).start()
    x_copy.start()
    wo_copy(0).start()

    def zero_body(i, carry):
        acc_ref[blk(i, T), :] = jnp.zeros((T, M), f32)
        return carry

    jax.lax.fori_loop(0, NB, zero_body, 0)
    bk_s[0:8, :] = jnp.zeros((8, T), u32)
    zm_s[...] = jnp.zeros((8, T), u32)
    for cp in kv_copies(0):
        cp.wait()
    wkv_s[:, :HP * D] = _pk(unpack_pair(rk_s[...]))
    wkv_s[:, HP * D:] = _pk(unpack_pair(rv_s[...]))
    for cp in kv_copies(1):
        cp.start()
    for cp in small:
        cp.wait()
    d_s[...] = dr_s[...].astype(f32)
    c_copy.wait()

    def gate_body(i, carry):
        gw = gw_s[...].astype(f32)
        xf = _upk(x_s[blk(i, T // 2), :]).astype(f32)
        t = xf[:, 0:T] * gw[0:1, :]
        for j in range(1, M // T):
            t = t + xf[:, j * T:(j + 1) * T] * gw[j:j + 1, :]
        z = jnp.sum(t, axis=-1, keepdims=True)
        g = 0.5 * jnp.tanh(0.5 * z) + 0.5
        g_s[blk(i, T), :] = jnp.broadcast_to(g, (T, T))
        return carry

    def loop_body(s, carry):
        @pl.when(s >= 0)
        def _():
            phase_b(s)

        @pl.when(s + 1 < NSTEP)
        def _():
            phase_a(s + 1)

        @pl.when(s < 0)
        def _():
            x_copy.wait()
            jax.lax.fori_loop(0, NB, gate_body, 0, unroll=8)
        return carry

    jax.lax.fori_loop(-1, NSTEP, loop_body, 0)
    for i in range(NB):
        o_copy(i).wait()


@jax.jit
def pallas_gated_mix__compressed_kv_cla__ssm_conv_h3__prompt_kernel(
    A_x: jax.Array,
    A_c_kv: jax.Array,
    A_w_q: jax.Array,
    A_w_uk: jax.Array,
    A_w_uv: jax.Array,
    A_w_o: jax.Array,
    B_q: jax.Array,
    B_k: jax.Array,
    B_v: jax.Array,
    B_shift_k: jax.Array,
    B_ssm_k: jax.Array,
    B_ssm_D: jax.Array,
    gate_w: jax.Array,
):
    del B_q
    tab = jnp.asarray(_dft_tables(), bf16)
    out = pl.pallas_call(
        _kernel,
        in_specs=[pl.BlockSpec(memory_space=pl.ANY)] * 13,
        out_specs=pl.BlockSpec(memory_space=pl.ANY),
        out_shape=jax.ShapeDtypeStruct((S, M), bf16),
        scratch_shapes=[
            pltpu.VMEM((S, M), f32),
            pltpu.VMEM((S // 2, M), u32),
            pltpu.VMEM((S // 2, DC), u32),
            pltpu.VMEM((M, D), u32),
            pltpu.VMEM((DC, D), u32),
            pltpu.VMEM((DC, D), u32),
            pltpu.VMEM((2, HP * D, M), bf16),
            pltpu.VMEM((S // 2 + 8, T), u32),
            pltpu.VMEM((S // 2, T), u32),
            pltpu.VMEM((T, S), bf16),
            pltpu.VMEM((KS, M), bf16),
            pltpu.VMEM((M // T, T), bf16),
            pltpu.VMEM((M // T, T), bf16),
            pltpu.VMEM((6, T, T), bf16),
            pltpu.VMEM((M // 2, HP * D), u32),
            pltpu.VMEM((DC // 2, 2 * HP * D), u32),
            pltpu.VMEM((S // 2, HP * D), u32),
            pltpu.VMEM((S // 2, HP * D), u32),
            pltpu.VMEM((S, T), f32),
            pltpu.VMEM((M // T, T), f32),
            pltpu.VMEM((S, M), bf16),
            pltpu.VMEM((S, T), f32),
            pltpu.VMEM((S, T), bf16),
            pltpu.VMEM((8, T), u32),
            pltpu.SemaphoreType.DMA((5,)),
            pltpu.SemaphoreType.DMA((2,)),
            pltpu.SemaphoreType.DMA((2,)),
            pltpu.SemaphoreType.DMA((4,)),
            pltpu.SemaphoreType.DMA(()),
        ],
        compiler_params=pltpu.CompilerParams(
            vmem_limit_bytes=100 * 1024 * 1024,
            disable_bounds_checks=True,
        ),
    )(
        A_x.reshape(S, M), A_c_kv.reshape(S, DC), A_w_q, A_w_uk, A_w_uv, A_w_o.reshape(H * D, M),
        B_k.reshape(S, M), B_v.reshape(S, M), B_shift_k.T, B_ssm_k,
        B_ssm_D.reshape(M // T, T), gate_w.reshape(M // T, T), tab,
    )
    return out.reshape(1, S, M)
```

```python
import functools

import jax
import jax.numpy as jnp
import numpy as np
import jax.experimental.pallas as pl
import jax.experimental.pallas.tpu as pltpu

f32 = jnp.float32
bf16 = jnp.bfloat16
u32 = jnp.uint32

S = 2048
M = 1024
H = 32
D = 128
DC = 512
T = 128
NB = S // T
NP = NB // 2
HP = 2
NSTEP = H // HP
HF = T // 2
KS = 4
LOG2E = 1.4426950408889634
NT = (((1,), (1,)), ((), ()))

G1, G2 = 2, 2
NUNP = 4
LAG = 5
WPU = 4


def _pk(v):
    return pltpu.bitcast(v, u32)


def _upk(v):
    return pltpu.bitcast(v, bf16)


def _hs(a, b):
    return slice(a // 2, b // 2)


def _lo(w):
    return pltpu.bitcast(w << 16, f32)


def _hi(w):
    return pltpu.bitcast(w & jnp.uint32(0xFFFF0000), f32)


def _dft_tables():
    n = np.arange(T)[None, :]
    fw, inv = [], []
    for half in range(2):
        f = (np.arange(HF) * 2 + half)[:, None]
        th = 2.0 * np.pi * (f + 0.5) * n / (2 * T)
        m = np.concatenate([np.cos(th), -np.sin(th)], axis=0)
        fw.append(m)
        inv.append(m.T / T)
    perm = np.concatenate([np.arange(0, T, 2), np.arange(1, T, 2)])
    fwp = [m[:, perm] for m in fw]
    return np.concatenate([np.stack(fw), np.stack(inv), np.stack(fwp)], axis=0).astype(np.float32)


def _lhs7(a11, a12, a21, a22):
    return [a11 + a22, a21 + a22, a11, a22, a11 + a12, a21 - a11, a12 - a22]


def _rhs7(b11, b12, b21, b22):
    return [b11 + b22, b11, b12 - b22, b21 - b11, b22, b11 + b12, b21 + b22]


def _comb(m):
    c11 = m[0] + m[3] - m[4] + m[6]
    c12 = m[2] + m[4]
    c21 = m[1] + m[3]
    c22 = m[0] - m[1] + m[2] + m[5]
    return c11, c12, c21, c22


_MORDER = [0, 3, 4, 6, 1, 2, 5]


def _kernel(x_hbm, c_hbm, wq_hbm, wk_hbm, wv_hbm, wo_hbm, bk_hbm, bv_hbm, sh_hbm, hk_hbm,
            d_hbm, gw_hbm, tab_hbm, o_hbm,
            acc_ref, x_s, c_s, x7_s, c7_s, rq_s, rk_s, rv_s, ro_s, bk_s, bv_s, hk_s, sh_s, dr_s, gw_s, tab_s,
            wq_s, wkv_s, wo_s, k_s, v_s, g_s, d_s, o_s, z_s, u_s, zm_s,
            sem_a, sem_kv, sem_xc, sem_small, sem_o):
    x32 = x_hbm.bitcast(u32)
    c32 = c_hbm.bitcast(u32)
    wq32 = wq_hbm.bitcast(u32)
    wk32 = wk_hbm.bitcast(u32)
    wv32 = wv_hbm.bitcast(u32)
    bk32 = bk_hbm.bitcast(u32)
    bv32 = bv_hbm.bitcast(u32)

    def blk(idx, size):
        if isinstance(idx, int):
            return pl.ds(idx * size, size)
        return pl.ds(pl.multiple_of(idx * size, size), size)

    def conv_copies(grp):
        return [
            pltpu.make_async_copy(hk_hbm.at[blk(grp, T), :], hk_s, sem_a.at[0]),
            pltpu.make_async_copy(bk32.at[:, blk(grp, T)], bk_s.at[pl.ds(8, S // 2), :], sem_a.at[1]),
            pltpu.make_async_copy(bv32.at[:, blk(grp, T)], bv_s, sem_a.at[2]),
        ]

    def q_copy(s):
        return pltpu.make_async_copy(wq32.at[:, s, :], rq_s, sem_a.at[3])

    def kvo_copies(s):
        return [
            pltpu.make_async_copy(wk32.at[:, s, :], rk_s, sem_kv.at[0]),
            pltpu.make_async_copy(wv32.at[:, s, :], rv_s, sem_kv.at[1]),
            pltpu.make_async_copy(wo_hbm.at[blk(s, HP * D), :], ro_s, sem_kv.at[2]),
        ]

    x_copies = [pltpu.make_async_copy(x32.at[pl.ds(j * (S // 4), S // 4), :], x_s.at[pl.ds(j * (S // 4), S // 4), :],
                                      sem_xc.at[2 * j]) for j in range(2)]
    c_copy = pltpu.make_async_copy(c32, c_s, sem_xc.at[1])
    small = [
        pltpu.make_async_copy(tab_hbm, tab_s, sem_small.at[0]),
        pltpu.make_async_copy(sh_hbm, sh_s, sem_small.at[1]),
        pltpu.make_async_copy(d_hbm, dr_s, sem_small.at[2]),
        pltpu.make_async_copy(gw_hbm, gw_s, sem_small.at[3]),
    ]

    def o_copy(b):
        r = pl.ds(b * 2 * T, 2 * T)
        return pltpu.make_async_copy(o_s.at[r, :], o_hbm.at[r, :], sem_o)

    scale = (D ** -0.5) * LOG2E

    J5 = {0: 0, 1: 1, 4: 2, 5: 3, 6: 4}

    def lhs_deps(raw, comb, j, b, ncol, deps, zmask):
        nr = HF
        if j == 2:
            ref, r0, c0 = raw, b * T, 0
        elif j == 3:
            ref, r0, c0 = raw, b * T + HF, ncol
        else:
            ref, r0, c0 = comb, J5[j] * (S // 4) + b * HF, 0
        if not deps:
            return ref[r0:r0 + nr, c0:c0 + ncol]
        ntile = (nr // 8) * (ncol // T)
        assert len(deps) <= ntile, (len(deps), ntile)
        pos = {(k * ntile) // len(deps): d for k, d in enumerate(deps)}
        rows = []
        for rg in range(nr // 8):
            tiles = []
            for kt in range(ncol // T):
                tl = ref[r0 + rg * 8:r0 + (rg + 1) * 8, c0 + kt * T:c0 + (kt + 1) * T]
                idx = rg * (ncol // T) + kt
                if idx in pos:
                    tl = tl | (pltpu.bitcast(pos[idx], u32) & zmask)
                tiles.append(tl)
            rows.append(jnp.concatenate(tiles, axis=1))
        return jnp.concatenate(rows, axis=0)

    def fold(ws):
        t = None
        for w in ws:
            for r in range(0, w.shape[0], 8):
                for c in range(0, w.shape[1], T):
                    p = w[r:r + 8, c:c + T]
                    t = p if t is None else t | p
        return t

    def wq_piece(r0):
        top = rq_s[r0:r0 + 16, :]
        bot = rq_s[M // 2 + r0:M // 2 + r0 + 16, :]
        rs = _rhs7(_lo(top), _hi(top), _lo(bot), _hi(bot))
        w = _pk(jnp.concatenate(rs, axis=1).astype(bf16))
        wq_s[r0 // 2:r0 // 2 + 8, :] = w
        return [fold([_pk(rs[5]), _pk(rs[6])])]

    def wkv_piece(r0):
        tk, bk_ = rk_s[r0:r0 + 16, :], rk_s[DC // 2 + r0:DC // 2 + r0 + 16, :]
        tv, bv_ = rv_s[r0:r0 + 16, :], rv_s[DC // 2 + r0:DC // 2 + r0 + 16, :]
        rk = _rhs7(_lo(tk), _hi(tk), _lo(bk_), _hi(bk_))
        rv = _rhs7(_lo(tv), _hi(tv), _lo(bv_), _hi(bv_))
        w = _pk(jnp.concatenate([z for j in range(7) for z in (rk[j], rv[j])], axis=1).astype(bf16))
        wkv_s[r0 // 2:r0 // 2 + 8, :] = w
        return [fold([_pk(rk[5]), _pk(rk[6])]), fold([_pk(rv[5]), _pk(rv[6])])]

    def wo_piece(sl, r0, c0):
        b11 = ro_s[r0:r0 + 16, c0:c0 + T].astype(f32)
        b12 = ro_s[r0:r0 + 16, M // 2 + c0:M // 2 + c0 + T].astype(f32)
        b21 = ro_s[D + r0:D + r0 + 16, c0:c0 + T].astype(f32)
        b22 = ro_s[D + r0:D + r0 + 16, M // 2 + c0:M // 2 + c0 + T].astype(f32)
        rs = _rhs7(b11, b12, b21, b22)
        w = _pk(jnp.concatenate(rs, axis=1).astype(bf16))
        base = (c0 // T) * HF + r0 // 2
        if isinstance(sl, int):
            wo_s[sl * 4 * HF + base:sl * 4 * HF + base + 8, :] = w
        else:
            wo_s[pl.ds(pl.multiple_of(sl * (4 * HF) + base, 8), 8), :] = w
        return [fold([_pk(rs[5]), _pk(rs[6])])]

    def phase_a(s):
        slot = s & 1
        grp = s >> 1

        @pl.when(slot == 0)
        def _():
            for cp in conv_copies(grp):
                cp.wait()
        q_copy(s).wait()

        sgn = (1 - 2 * slot).astype(f32)
        zmask = zm_s[...]
        taps = sh_s[:, blk(grp, T)].astype(f32)
        dvec = d_s[pl.ds(grp, 1), :]
        hs = {}
        ab = {}
        k1 = {}
        ms = {}

        def projkv_u(b, j, deps):
            lhs = lhs_deps(c_s, c7_s, j, b, DC // 2, deps, zmask)
            m = jnp.dot(_upk(lhs), _upk(wkv_s[:, j * 2 * T:(j + 1) * 2 * T]), preferred_element_type=f32)
            ms[j] = m
            r1 = _hs(2 * b * T, (2 * b + 1) * T)
            r2 = _hs((2 * b + 1) * T, (2 * b + 2) * T)
            done = {6: (lambda: ms[0] + ms[3] - ms[4] + ms[6], r1, 0),
                    1: (lambda: ms[1] + ms[3], r2, 0),
                    2: (lambda: ms[2] + ms[4], r1, 1),
                    5: (lambda: ms[0] - ms[1] + ms[2] + ms[5], r2, 1)}
            if j in done:
                fn, r, hh = done[j]
                cc = fn()
                k_s[r, hh * T:(hh + 1) * T] = _pk(cc[:, :T].astype(bf16))
                v_s[r, hh * T:(hh + 1) * T] = _pk(cc[:, T:].astype(bf16))
            return pltpu.bitcast(m[0:8, 0:T], u32) & zmask

        def conv_h(m):
            hm = jax.lax.dot_general(tab_s[slot], hk_s[:, m * T:(m + 1) * T], NT,
                                     preferred_element_type=f32)
            hr, hi = hm[:HF], hm[HF:]
            if m == 0:
                hr = hr + dvec
            hs[m] = (hr, hi)
            if m > 0:
                pr, pi = hs[m - 1]
                hr = hr - sgn * pi
                hi = hi + sgn * pr
            ab[(0, m)] = hr
            ab[(1, m)] = hr + hi
            ab[(2, m)] = hi - hr

        def conv_prep(c):
            t0, t1, t2, t3 = [taps[j:j + 1, :] for j in range(KS)]
            deps = []
            for q in range(T // 32):
                r0 = c * HF + q * 16
                w0 = bk_s[8 + r0:8 + r0 + 16, :]
                w1 = bk_s[7 + r0:7 + r0 + 16, :]
                w2 = bk_s[6 + r0:6 + r0 + 16, :]
                e0, o0, e1, o1, o2 = _lo(w0), _hi(w0), _lo(w1), _hi(w1), _hi(w2)
                wv = bv_s[r0:r0 + 16, :]
                kve = (e0 * t0 + o1 * t1 + e1 * t2 + o2 * t3) * _lo(wv)
                kvo = (o0 * t0 + e0 * t1 + o1 * t2 + e1 * t3) * _hi(wv)
                u_s[c * T + q * 16:c * T + (q + 1) * 16, :] = kve.astype(bf16)
                u_s[c * T + HF + q * 16:c * T + HF + (q + 1) * 16, :] = kvo.astype(bf16)
                deps.append(kve[0:8] + kvo[0:8])
                deps.append(kve[8:16] + kvo[8:16])
            return deps

        def conv_u(c):
            u = jnp.dot(tab_s[4 + slot], u_s[c * T:(c + 1) * T, :], preferred_element_type=f32)
            ab[(4, c)] = u[HF:]
            ab[(5, c)] = u[:HF]

        def gated(v, tok):
            return pltpu.bitcast(pltpu.bitcast(v, u32) | tok, f32)

        def conv_mac(ty, p0, tok):
            sl = slice(p0, p0 + 8)
            a_ = [ab[(ty, m)][sl] for m in range(NB)]
            if ty == 0:
                b_ = [gated(ab[(5, c)][sl], tok) + ab[(4, c)][sl] for c in range(NB)]
            else:
                b_ = [gated(ab[(3 + ty, c)][sl], tok) for c in range(NB)]
            deps = []
            for a in range(NB):
                t = a_[a] * b_[0]
                for c in range(1, a + 1):
                    t = t + a_[a - c] * b_[c]
                if ty == 0:
                    k1[(a, p0)] = t
                elif ty == 1:
                    t = k1[(a, p0)] - t
                    z_s[a * T + p0:a * T + p0 + 8, :] = t
                else:
                    t = k1[(a, p0)] + t
                    z_s[a * T + HF + p0:a * T + HF + p0 + 8, :] = t
                deps.append(t)
            return deps

        units = [(b, j) for b in range(NP) for j in _MORDER]
        projkv_u(*units.pop(0), [])
        for m in range(NB):
            conv_h(m)
        chunks = [(ty, p0) for p0 in range(0, HF, 8) for ty in range(3)]
        q0 = NB + G1 + G2
        nmb = len(units) - q0 - NUNP
        start = [q0 - 1 + (j * (nmb - LAG)) // len(chunks) for j in range(len(chunks))]
        pend = {}
        nq = M // 2 // 16
        for k, (b, j) in enumerate(units):
            deps = pend.pop(k, [])
            if k < NB:
                deps = conv_prep(k)
            elif k >= q0 + nmb:
                kk = k - q0 - nmb
                for t in range(kk * nq // NUNP, (kk + 1) * nq // NUNP):
                    deps += wq_piece(t * 16)
            tok = projkv_u(b, j, deps)
            for jj, st in enumerate(start):
                if st == k:
                    pend.setdefault(k + LAG + 1, []).extend(conv_mac(*chunks[jj], tok))
            if k == NB + G1 - 1:
                for c in range(NB):
                    conv_u(c)
        assert not pend

    def phase_b(s):
        slot = s & 1
        grp = s >> 1
        cols = blk(grp, T)

        @pl.when(s + 1 < NSTEP)
        def _():
            q_copy(s + 1).start()

        @pl.when(jnp.logical_and(s + 1 < NSTEP, slot == 1))
        def _():
            for cp in conv_copies(grp + 1):
                cp.start()

        @pl.when(s + 1 < NSTEP)
        def _():
            for cp in kvo_copies(s + 1):
                cp.wait()

        row = jax.lax.broadcasted_iota(jnp.int32, (T, T), 0)
        col = jax.lax.broadcasted_iota(jnp.int32, (T, T), 1)
        tri = col <= row
        zmask = zm_s[...]
        qh = {}

        wwork = ([functools.partial(wo_piece, 1 - slot, r0, c0) for c0 in range(0, M // 2, T)
                  for r0 in range(0, D, 16)]
                 + [functools.partial(wkv_piece, r0) for r0 in range(0, DC // 2, 16)])
        qms = {}

        def projq(b, hf):
            ms = qms.setdefault(b, {})
            for j in (_MORDER[:4] if hf == 0 else _MORDER[4:]):
                deps = []
                for _ in range(WPU):
                    if wwork:
                        deps += wwork.pop(0)()
                        if not wwork:
                            @pl.when(s + 2 < NSTEP)
                            def _():
                                for cp in kvo_copies(s + 2):
                                    cp.start()
                lhs = lhs_deps(x_s, x7_s, j, b, M // 2, deps, zmask)
                ms[j] = jnp.dot(_upk(lhs), _upk(wq_s[:, j * T:(j + 1) * T]), preferred_element_type=f32)
            if hf == 1:
                c11, c12, c21, c22 = _comb(ms)
                qh[(2 * b, 0)] = c11 * scale
                qh[(2 * b, 1)] = c12 * scale
                qh[(2 * b + 1, 0)] = c21 * scale
                qh[(2 * b + 1, 1)] = c22 * scale

        def scores(i, hh):
            cs = slice(hh * D, (hh + 1) * D)
            return jax.lax.dot_general(qh[(i, hh)].astype(bf16), _upk(k_s[_hs(0, (i + 1) * T), cs]), NT,
                                       preferred_element_type=f32)

        def softmax(i, sc):
            base = i * T
            dg = jnp.where(tri, sc[:, base:], -1e30)
            srow = jnp.concatenate([sc[:, :base], dg], axis=1) if base > 0 else dg
            m = jnp.max(srow, axis=-1, keepdims=True)
            p = jnp.exp2(srow - m)
            l = jnp.sum(p, axis=-1, keepdims=True)
            r = pl.reciprocal(l, approx=True)
            r = r * (2.0 - l * r)
            return p, g_s[base:base + T, :] * r

        def pv(i, hh, p, sc):
            cs = slice(hh * D, (hh + 1) * D)
            return jnp.dot(p.astype(bf16), _upk(v_s[_hs(0, (i + 1) * T), cs]),
                           preferred_element_type=f32) * sc

        def conv_inv(a):
            r = slice(a * T, (a + 1) * T)
            y = jnp.dot(tab_s[2 + slot], z_s[r, :].astype(bf16), preferred_element_type=f32)
            xc = _upk(x_s[_hs(a * T, (a + 1) * T), cols]).astype(f32)
            acc_ref[r, cols] += y * xc * (1.0 - g_s[r, :])

        ctx = {}
        ls = {}

        def outp(b, hf):
            if hf == 0:
                ls[b] = [l.astype(bf16) for l in _lhs7(ctx[(2 * b, 0)], ctx[(2 * b, 1)],
                                                       ctx[(2 * b + 1, 0)], ctx[(2 * b + 1, 1)])]
            r1 = slice(2 * b * T, (2 * b + 1) * T)
            r2 = slice((2 * b + 1) * T, (2 * b + 2) * T)
            parts = []
            for ct in range(2 * hf, 2 * hf + 2):
                ms = {}
                for j in _MORDER:
                    ms[j] = jnp.dot(ls[b][j], _upk(wo_s[pl.ds(pl.multiple_of(slot * (4 * HF) + ct * HF, HF), HF), j * T:(j + 1) * T]),
                                    preferred_element_type=f32)
                parts.append(_comb(ms))
            ca = slice(2 * hf * T, (2 * hf + 2) * T)
            cb = slice(M // 2 + 2 * hf * T, M // 2 + (2 * hf + 2) * T)
            for n, (r, c) in enumerate(((r1, ca), (r1, cb), (r2, ca), (r2, cb))):
                res = acc_ref[r, c] + jnp.concatenate([parts[0][n], parts[1][n]], axis=1)
                acc_ref[r, c] = res
                o_s[r, c] = res.astype(bf16)
            if hf == 1:
                @pl.when(s == NSTEP - 1)
                def _():
                    o_copy(b).start()

        order = list(range(NB - 1, -1, -1))
        projq(NP - 1, 0)
        projq(NP - 1, 1)
        qtodo = [(b, hf) for b in range(NP - 2, -1, -1) for hf in range(2)]
        otodo = []
        for i in order:
            ss = [scores(i, hh) for hh in range(HP)]
            fill = []
            if qtodo:
                fill.append(functools.partial(projq, *qtodo.pop(0)))
            if otodo:
                fill.append(functools.partial(outp, *otodo.pop(0)))
            for hh in range(HP):
                p, sc = softmax(i, ss[hh])
                if fill:
                    fill.pop(0)()
                ctx[(i, hh)] = pv(i, hh, p, sc)
            conv_inv(i)
            for fn in fill:
                fn()
            if i % 2 == 0:
                otodo += [(i // 2, 0), (i // 2, 1)]
        for a in otodo:
            outp(*a)
        assert not wwork

    kvo0 = kvo_copies(0)
    kvo0[0].start()
    kvo0[1].start()
    for cp in small:
        cp.start()
    c_copy.start()
    for cp in conv_copies(0):
        cp.start()
    q_copy(0).start()
    x_copies[0].start()
    kvo0[2].start()
    x_copies[1].start()

    def zero_body(i, carry):
        acc_ref[blk(i, T), :] = jnp.zeros((T, M), f32)
        return carry

    jax.lax.fori_loop(0, NB, zero_body, 0)
    bk_s[0:8, :] = jnp.zeros((8, T), u32)
    zm_s[...] = jnp.zeros((8, T), u32)
    kvo0[0].wait()
    kvo0[1].wait()
    for r0 in range(0, DC // 2, 16):
        wkv_piece(r0)
    kvo1 = kvo_copies(1)
    kvo1[0].start()
    kvo1[1].start()
    for cp in small:
        cp.wait()
    d_s[...] = dr_s[...].astype(f32)
    c_copy.wait()

    def comb_rows(src, dst, b, r0, nr, ncol):
        w1 = src[b * T + r0:b * T + r0 + nr, :]
        w2 = src[b * T + HF + r0:b * T + HF + r0 + nr, :]
        a1 = _upk(w1).astype(f32)
        a2 = _upk(w2).astype(f32)
        h = ncol // 2
        l7 = _lhs7(a1[:, :h], a1[:, h:], a2[:, :h], a2[:, h:])
        for j, jj in J5.items():
            rr = slice(jj * (S // 4) + b * HF + r0, jj * (S // 4) + b * HF + r0 + nr)
            dst[rr, :] = _pk(l7[j].astype(bf16))
        return a1, a2

    for b in range(NP):
        for r0 in range(0, HF, 8):
            comb_rows(c_s, c7_s, b, r0, 8, DC)

    def x_prep(b0, b1):
        gw = gw_s[...].astype(f32)
        for b in range(b0, b1):
            for r0 in range(0, HF, 8):
                rows = comb_rows(x_s, x7_s, b, r0, 8, M)
                for half, xf in enumerate(rows):
                    t = xf[:, 0:T] * gw[0:1, :]
                    for j in range(1, M // T):
                        t = t + xf[:, j * T:(j + 1) * T] * gw[j:j + 1, :]
                    z = jnp.sum(t, axis=-1, keepdims=True)
                    g = 0.5 * jnp.tanh(0.5 * z) + 0.5
                    g0 = b * 2 * T + half * T + 2 * r0
                    g_s[g0:g0 + 16, :] = jnp.broadcast_to(g, (16, T))

    def loop_body(s, carry):
        @pl.when(s >= 0)
        def _():
            phase_b(s)

        @pl.when(s + 1 < NSTEP)
        def _():
            phase_a(s + 1)

        @pl.when(s < 0)
        def _():
            kvo0[2].wait()
            for c0 in range(0, M // 2, T):
                for r0 in range(0, D, 16):
                    wo_piece(0, r0, c0)
            kvo1[2].start()
            x_copies[0].wait()
            x_prep(0, NP // 2)
            x_copies[1].wait()
            x_prep(NP // 2, NP)
        return carry

    jax.lax.fori_loop(-1, NSTEP, loop_body, 0)
    for b in range(NP):
        o_copy(b).wait()


@jax.jit
def pallas_gated_mix__compressed_kv_cla__ssm_conv_h3__prompt_kernel(
    A_x, A_c_kv, A_w_q, A_w_uk, A_w_uv, A_w_o, B_q, B_k, B_v, B_shift_k, B_ssm_k, B_ssm_D, gate_w,
):
    del B_q
    tab = jnp.asarray(_dft_tables(), bf16)
    out = pl.pallas_call(
        _kernel,
        in_specs=[pl.BlockSpec(memory_space=pl.ANY)] * 13,
        out_specs=pl.BlockSpec(memory_space=pl.ANY),
        out_shape=jax.ShapeDtypeStruct((S, M), bf16),
        scratch_shapes=[
            pltpu.VMEM((S, M), f32),
            pltpu.VMEM((S // 2, M), u32),
            pltpu.VMEM((S // 2, DC), u32),
            pltpu.VMEM((5 * S // 4, M // 2), u32),
            pltpu.VMEM((5 * S // 4, DC // 2), u32),
            pltpu.VMEM((M, D), u32),
            pltpu.VMEM((DC, D), u32),
            pltpu.VMEM((DC, D), u32),
            pltpu.VMEM((HP * D, M), bf16),
            pltpu.VMEM((S // 2 + 8, T), u32),
            pltpu.VMEM((S // 2, T), u32),
            pltpu.VMEM((T, S), bf16),
            pltpu.VMEM((KS, M), bf16),
            pltpu.VMEM((M // T, T), bf16),
            pltpu.VMEM((M // T, T), bf16),
            pltpu.VMEM((6, T, T), bf16),
            pltpu.VMEM((M // 4, 7 * T), u32),
            pltpu.VMEM((DC // 4, 14 * T), u32),
            pltpu.VMEM((2 * 4 * HF, 7 * T), u32),
            pltpu.VMEM((S // 2, HP * D), u32),
            pltpu.VMEM((S // 2, HP * D), u32),
            pltpu.VMEM((S, T), f32),
            pltpu.VMEM((M // T, T), f32),
            pltpu.VMEM((S, M), bf16),
            pltpu.VMEM((S, T), f32),
            pltpu.VMEM((S, T), bf16),
            pltpu.VMEM((8, T), u32),
            pltpu.SemaphoreType.DMA((4,)),
            pltpu.SemaphoreType.DMA((3,)),
            pltpu.SemaphoreType.DMA((3,)),
            pltpu.SemaphoreType.DMA((4,)),
            pltpu.SemaphoreType.DMA(()),
        ],
        compiler_params=pltpu.CompilerParams(
            vmem_limit_bytes=100 * 1024 * 1024,
            disable_bounds_checks=True,
        ),
    )(
        A_x.reshape(S, M), A_c_kv.reshape(S, DC), A_w_q, A_w_uk, A_w_uv, A_w_o.reshape(H * D, M),
        B_k.reshape(S, M), B_v.reshape(S, M), B_shift_k.T, B_ssm_k,
        B_ssm_D.reshape(M // T, T), gate_w.reshape(M // T, T), tab,
    )
    return out.reshape(1, S, M)
```

```python
import functools

import jax
import jax.numpy as jnp
import numpy as np
import jax.experimental.pallas as pl
import jax.experimental.pallas.tpu as pltpu

f32 = jnp.float32
bf16 = jnp.bfloat16
u32 = jnp.uint32

S = 2048
M = 1024
H = 32
D = 128
DC = 512
T = 128
NB = S // T
NP = NB // 2
HP = 2
NSTEP = H // HP
HF = T // 2
KS = 4
LOG2E = 1.4426950408889634
NT = (((1,), (1,)), ((), ()))

G1, G2 = 2, 2
NUNP = 4
LAG = 5
WPU = 4


def _pk(v):
    return pltpu.bitcast(v, u32)


def _upk(v):
    return pltpu.bitcast(v, bf16)


def _hs(a, b):
    return slice(a // 2, b // 2)


def _lo(w):
    return pltpu.bitcast(w << 16, f32)


def _hi(w):
    return pltpu.bitcast(w & jnp.uint32(0xFFFF0000), f32)


def _dft_tables():
    n = np.arange(T)[None, :]
    fw, inv = [], []
    for half in range(2):
        f = (np.arange(HF) * 2 + half)[:, None]
        th = 2.0 * np.pi * (f + 0.5) * n / (2 * T)
        m = np.concatenate([np.cos(th), -np.sin(th)], axis=0)
        fw.append(m)
        inv.append(m.T / T)
    perm = np.concatenate([np.arange(0, T, 2), np.arange(1, T, 2)])
    fwp = [m[:, perm] for m in fw]
    return np.concatenate([np.stack(fw), np.stack(inv), np.stack(fwp)], axis=0).astype(np.float32)


def _lhs7(a11, a12, a21, a22):
    return [a11 + a22, a21 + a22, a11, a22, a11 + a12, a21 - a11, a12 - a22]


def _rhs7(b11, b12, b21, b22):
    return [b11 + b22, b11, b12 - b22, b21 - b11, b22, b11 + b12, b21 + b22]


def _comb(m):
    c11 = m[0] + m[3] - m[4] + m[6]
    c12 = m[2] + m[4]
    c21 = m[1] + m[3]
    c22 = m[0] - m[1] + m[2] + m[5]
    return c11, c12, c21, c22


_MORDER = [0, 3, 4, 6, 1, 2, 5]


def _kernel(x_hbm, c_hbm, wq_hbm, wk_hbm, wv_hbm, wo_hbm, bk_hbm, bv_hbm, sh_hbm, hk_hbm,
            d_hbm, gw_hbm, tab_hbm, o_hbm,
            acc_ref, x_s, c_s, x7_s, c7_s, rq_s, rk_s, rv_s, ro_s, bk_s, bv_s, hk_s, sh_s, dr_s, gw_s, tab_s,
            wq_s, wkv_s, wo_s, k_s, v_s, g_s, d_s, o_s, z_s, u_s, zm_s,
            sem_a, sem_kv, sem_xc, sem_small, sem_o):
    x32 = x_hbm.bitcast(u32)
    c32 = c_hbm.bitcast(u32)
    wq32 = wq_hbm.bitcast(u32)
    wk32 = wk_hbm.bitcast(u32)
    wv32 = wv_hbm.bitcast(u32)
    bk32 = bk_hbm.bitcast(u32)
    bv32 = bv_hbm.bitcast(u32)

    def blk(idx, size):
        if isinstance(idx, int):
            return pl.ds(idx * size, size)
        return pl.ds(pl.multiple_of(idx * size, size), size)

    def conv_copies(grp):
        return [
            pltpu.make_async_copy(hk_hbm.at[blk(grp, T), :], hk_s, sem_a.at[0]),
            pltpu.make_async_copy(bk32.at[:, blk(grp, T)], bk_s.at[pl.ds(8, S // 2), :], sem_a.at[1]),
            pltpu.make_async_copy(bv32.at[:, blk(grp, T)], bv_s, sem_a.at[2]),
        ]

    def q_copy(s):
        return pltpu.make_async_copy(wq32.at[:, s, :], rq_s, sem_a.at[3])

    def kvo_copies(s):
        return [
            pltpu.make_async_copy(wk32.at[:, s, :], rk_s, sem_kv.at[0]),
            pltpu.make_async_copy(wv32.at[:, s, :], rv_s, sem_kv.at[1]),
            pltpu.make_async_copy(wo_hbm.at[blk(s, HP * D), :], ro_s, sem_kv.at[2]),
        ]

    x_copies = [pltpu.make_async_copy(x32.at[pl.ds(j * (S // 4), S // 4), :], x_s.at[pl.ds(j * (S // 4), S // 4), :],
                                      sem_xc.at[2 * j]) for j in range(2)]
    c_copy = pltpu.make_async_copy(c32, c_s, sem_xc.at[1])
    small = [
        pltpu.make_async_copy(tab_hbm, tab_s, sem_small.at[0]),
        pltpu.make_async_copy(sh_hbm, sh_s, sem_small.at[1]),
        pltpu.make_async_copy(d_hbm, dr_s, sem_small.at[2]),
        pltpu.make_async_copy(gw_hbm, gw_s, sem_small.at[3]),
    ]

    def o_copy(b):
        r = pl.ds(b * 2 * T, 2 * T)
        return pltpu.make_async_copy(o_s.at[r, :], o_hbm.at[r, :], sem_o)

    scale = (D ** -0.5) * LOG2E

    J5 = {0: 0, 1: 1, 4: 2, 5: 3, 6: 4}

    def lhs_deps(raw, comb, j, b, ncol, deps, zmask):
        nr = HF
        if j == 2:
            ref, r0, c0 = raw, b * T, 0
        elif j == 3:
            ref, r0, c0 = raw, b * T + HF, ncol
        else:
            ref, r0, c0 = comb, J5[j] * (S // 4) + b * HF, 0
        if not deps:
            return ref[r0:r0 + nr, c0:c0 + ncol]
        ntile = (nr // 8) * (ncol // T)
        assert len(deps) <= ntile, (len(deps), ntile)
        pos = {(k * ntile) // len(deps): d for k, d in enumerate(deps)}
        rows = []
        for rg in range(nr // 8):
            tiles = []
            for kt in range(ncol // T):
                tl = ref[r0 + rg * 8:r0 + (rg + 1) * 8, c0 + kt * T:c0 + (kt + 1) * T]
                idx = rg * (ncol // T) + kt
                if idx in pos:
                    tl = tl | (pltpu.bitcast(pos[idx], u32) & zmask)
                tiles.append(tl)
            rows.append(jnp.concatenate(tiles, axis=1))
        return jnp.concatenate(rows, axis=0)

    def fold(ws):
        t = None
        for w in ws:
            for r in range(0, w.shape[0], 8):
                for c in range(0, w.shape[1], T):
                    p = w[r:r + 8, c:c + T]
                    t = p if t is None else t | p
        return t

    def wq_piece(r0):
        top = rq_s[r0:r0 + 16, :]
        bot = rq_s[M // 2 + r0:M // 2 + r0 + 16, :]
        rs = _rhs7(_lo(top), _hi(top), _lo(bot), _hi(bot))
        w = _pk(jnp.concatenate(rs, axis=1).astype(bf16))
        wq_s[r0 // 2:r0 // 2 + 8, :] = w
        return [fold([_pk(rs[5]), _pk(rs[6])])]

    def wkv_piece(r0):
        tk, bk_ = rk_s[r0:r0 + 16, :], rk_s[DC // 2 + r0:DC // 2 + r0 + 16, :]
        tv, bv_ = rv_s[r0:r0 + 16, :], rv_s[DC // 2 + r0:DC // 2 + r0 + 16, :]
        rk = _rhs7(_lo(tk), _hi(tk), _lo(bk_), _hi(bk_))
        rv = _rhs7(_lo(tv), _hi(tv), _lo(bv_), _hi(bv_))
        w = _pk(jnp.concatenate([z for j in range(7) for z in (rk[j], rv[j])], axis=1).astype(bf16))
        wkv_s[r0 // 2:r0 // 2 + 8, :] = w
        return [fold([_pk(rk[5]), _pk(rk[6])]), fold([_pk(rv[5]), _pk(rv[6])])]

    def wo_piece(sl, r0, c0):
        b11 = ro_s[r0:r0 + 16, c0:c0 + T].astype(f32)
        b12 = ro_s[r0:r0 + 16, M // 2 + c0:M // 2 + c0 + T].astype(f32)
        b21 = ro_s[D + r0:D + r0 + 16, c0:c0 + T].astype(f32)
        b22 = ro_s[D + r0:D + r0 + 16, M // 2 + c0:M // 2 + c0 + T].astype(f32)
        rs = _rhs7(b11, b12, b21, b22)
        w = _pk(jnp.concatenate(rs, axis=1).astype(bf16))
        base = (c0 // T) * HF + r0 // 2
        if isinstance(sl, int):
            wo_s[sl * 4 * HF + base:sl * 4 * HF + base + 8, :] = w
        else:
            wo_s[pl.ds(pl.multiple_of(sl * (4 * HF) + base, 8), 8), :] = w
        return [fold([_pk(rs[5]), _pk(rs[6])])]

    def phase_a(s):
        slot = s & 1
        grp = s >> 1

        @pl.when(slot == 0)
        def _():
            for cp in conv_copies(grp):
                cp.wait()
        q_copy(s).wait()

        sgn = (1 - 2 * slot).astype(f32)
        zmask = zm_s[...]
        taps = sh_s[:, blk(grp, T)].astype(f32)
        dvec = d_s[pl.ds(grp, 1), :]
        hs = {}
        ab = {}
        k1 = {}
        ms = {}

        def projkv_u(b, j, deps):
            lhs = lhs_deps(c_s, c7_s, j, b, DC // 2, deps, zmask)
            m = jnp.dot(_upk(lhs), _upk(wkv_s[:, j * 2 * T:(j + 1) * 2 * T]), preferred_element_type=f32)
            ms[j] = m
            r1 = _hs(2 * b * T, (2 * b + 1) * T)
            r2 = _hs((2 * b + 1) * T, (2 * b + 2) * T)
            done = {6: (lambda: ms[0] + ms[3] - ms[4] + ms[6], r1, 0),
                    1: (lambda: ms[1] + ms[3], r2, 0),
                    2: (lambda: ms[2] + ms[4], r1, 1),
                    5: (lambda: ms[0] - ms[1] + ms[2] + ms[5], r2, 1)}
            if j in done:
                fn, r, hh = done[j]
                cc = fn()
                k_s[r, hh * T:(hh + 1) * T] = _pk(cc[:, :T].astype(bf16))
                v_s[r, hh * T:(hh + 1) * T] = _pk(cc[:, T:].astype(bf16))
            return pltpu.bitcast(m[0:8, 0:T], u32) & zmask

        def conv_h(m):
            hm = jax.lax.dot_general(tab_s[slot], hk_s[:, m * T:(m + 1) * T], NT,
                                     preferred_element_type=f32)
            hr, hi = hm[:HF], hm[HF:]
            if m == 0:
                hr = hr + dvec
            hs[m] = (hr, hi)
            if m > 0:
                pr, pi = hs[m - 1]
                hr = hr - sgn * pi
                hi = hi + sgn * pr
            ab[(0, m)] = hr
            ab[(1, m)] = hr + hi
            ab[(2, m)] = hi - hr

        def conv_prep(c):
            t0, t1, t2, t3 = [taps[j:j + 1, :] for j in range(KS)]
            deps = []
            for q in range(T // 32):
                r0 = c * HF + q * 16
                w0 = bk_s[8 + r0:8 + r0 + 16, :]
                w1 = bk_s[7 + r0:7 + r0 + 16, :]
                w2 = bk_s[6 + r0:6 + r0 + 16, :]
                e0, o0, e1, o1, o2 = _lo(w0), _hi(w0), _lo(w1), _hi(w1), _hi(w2)
                wv = bv_s[r0:r0 + 16, :]
                kve = (e0 * t0 + o1 * t1 + e1 * t2 + o2 * t3) * _lo(wv)
                kvo = (o0 * t0 + e0 * t1 + o1 * t2 + e1 * t3) * _hi(wv)
                u_s[c * T + q * 16:c * T + (q + 1) * 16, :] = kve.astype(bf16)
                u_s[c * T + HF + q * 16:c * T + HF + (q + 1) * 16, :] = kvo.astype(bf16)
                deps.append(kve[0:8] + kvo[0:8])
                deps.append(kve[8:16] + kvo[8:16])
            return deps

        def conv_u(c):
            u = jnp.dot(tab_s[4 + slot], u_s[c * T:(c + 1) * T, :], preferred_element_type=f32)
            ab[(4, c)] = u[HF:]
            ab[(5, c)] = u[:HF]

        def gated(v, tok):
            return pltpu.bitcast(pltpu.bitcast(v, u32) | tok, f32)

        def conv_mac(ty, p0, tok):
            sl = slice(p0, p0 + 8)
            a_ = [ab[(ty, m)][sl] for m in range(NB)]
            if ty == 0:
                b_ = [gated(ab[(5, c)][sl], tok) + ab[(4, c)][sl] for c in range(NB)]
            else:
                b_ = [gated(ab[(3 + ty, c)][sl], tok) for c in range(NB)]
            deps = []
            for a in range(NB):
                t = a_[a] * b_[0]
                for c in range(1, a + 1):
                    t = t + a_[a - c] * b_[c]
                if ty == 0:
                    k1[(a, p0)] = t
                elif ty == 1:
                    t = k1[(a, p0)] - t
                    z_s[a * T + p0:a * T + p0 + 8, :] = t
                else:
                    t = k1[(a, p0)] + t
                    z_s[a * T + HF + p0:a * T + HF + p0 + 8, :] = t
                deps.append(t)
            return deps

        units = [(b, j) for b in range(NP) for j in _MORDER]
        projkv_u(*units.pop(0), [])
        for m in range(NB):
            conv_h(m)
        chunks = [(ty, p0) for p0 in range(0, HF, 8) for ty in range(3)]
        q0 = NB + G1 + G2
        nmb = len(units) - q0 - NUNP
        start = [q0 - 1 + (j * (nmb - LAG)) // len(chunks) for j in range(len(chunks))]
        pend = {}
        nq = M // 2 // 16
        for k, (b, j) in enumerate(units):
            deps = pend.pop(k, [])
            if k < NB:
                deps = conv_prep(k)
            elif k >= q0 + nmb:
                kk = k - q0 - nmb
                for t in range(kk * nq // NUNP, (kk + 1) * nq // NUNP):
                    deps += wq_piece(t * 16)
            tok = projkv_u(b, j, deps)
            for jj, st in enumerate(start):
                if st == k:
                    pend.setdefault(k + LAG + 1, []).extend(conv_mac(*chunks[jj], tok))
            if k == NB + G1 - 1:
                for c in range(NB):
                    conv_u(c)
        assert not pend

    def phase_b(s):
        slot = s & 1
        grp = s >> 1
        cols = blk(grp, T)

        @pl.when(s + 1 < NSTEP)
        def _():
            q_copy(s + 1).start()

        @pl.when(jnp.logical_and(s + 1 < NSTEP, slot == 1))
        def _():
            for cp in conv_copies(grp + 1):
                cp.start()

        @pl.when(s + 1 < NSTEP)
        def _():
            for cp in kvo_copies(s + 1):
                cp.wait()

        row = jax.lax.broadcasted_iota(jnp.int32, (T, T), 0)
        col = jax.lax.broadcasted_iota(jnp.int32, (T, T), 1)
        tri = col <= row
        zmask = zm_s[...]
        qh = {}

        wwork = ([functools.partial(wo_piece, 1 - slot, r0, c0) for c0 in range(0, M // 2, T)
                  for r0 in range(0, D, 16)]
                 + [functools.partial(wkv_piece, r0) for r0 in range(0, DC // 2, 16)])
        qms = {}

        def projq(b, hf):
            ms = qms.setdefault(b, {})
            for j in (_MORDER[:4] if hf == 0 else _MORDER[4:]):
                deps = []
                for _ in range(WPU):
                    if wwork:
                        deps += wwork.pop(0)()
                        if not wwork:
                            @pl.when(s + 2 < NSTEP)
                            def _():
                                for cp in kvo_copies(s + 2):
                                    cp.start()
                lhs = lhs_deps(x_s, x7_s, j, b, M // 2, deps, zmask)
                ms[j] = jnp.dot(_upk(lhs), _upk(wq_s[:, j * T:(j + 1) * T]), preferred_element_type=f32)
            if hf == 1:
                c11, c12, c21, c22 = _comb(ms)
                qh[(2 * b, 0)] = c11 * scale
                qh[(2 * b, 1)] = c12 * scale
                qh[(2 * b + 1, 0)] = c21 * scale
                qh[(2 * b + 1, 1)] = c22 * scale

        def scores(i, hh):
            cs = slice(hh * D, (hh + 1) * D)
            return jax.lax.dot_general(qh[(i, hh)].astype(bf16), _upk(k_s[_hs(0, (i + 1) * T), cs]), NT,
                                       preferred_element_type=f32)

        def softmax(i, sc):
            base = i * T
            dg = jnp.where(tri, sc[:, base:], -1e30)
            srow = jnp.concatenate([sc[:, :base], dg], axis=1) if base > 0 else dg
            m = jnp.max(srow, axis=-1, keepdims=True)
            p = jnp.exp2(srow - m)
            l = jnp.sum(p, axis=-1, keepdims=True)
            r = pl.reciprocal(l, approx=True)
            r = r * (2.0 - l * r)
            return p, g_s[base:base + T, :] * r

        def pv(i, hh, p, sc):
            cs = slice(hh * D, (hh + 1) * D)
            return jnp.dot(p.astype(bf16), _upk(v_s[_hs(0, (i + 1) * T), cs]),
                           preferred_element_type=f32) * sc

        def conv_inv(a):
            r = slice(a * T, (a + 1) * T)
            y = jnp.dot(tab_s[2 + slot], z_s[r, :].astype(bf16), preferred_element_type=f32)
            xc = _upk(x_s[_hs(a * T, (a + 1) * T), cols]).astype(f32)
            acc_ref[r, cols] += y * xc * (1.0 - g_s[r, :])

        ctx = {}
        ls = {}

        def outp(b, hf):
            if hf == 0:
                ls[b] = [l.astype(bf16) for l in _lhs7(ctx[(2 * b, 0)], ctx[(2 * b, 1)],
                                                       ctx[(2 * b + 1, 0)], ctx[(2 * b + 1, 1)])]
            r1 = slice(2 * b * T, (2 * b + 1) * T)
            r2 = slice((2 * b + 1) * T, (2 * b + 2) * T)
            parts = []
            for ct in range(2 * hf, 2 * hf + 2):
                ms = {}
                for j in _MORDER:
                    ms[j] = jnp.dot(ls[b][j], _upk(wo_s[blk(slot * 4 + ct, HF), j * T:(j + 1) * T]),
                                    preferred_element_type=f32)
                parts.append(_comb(ms))
            ca = slice(2 * hf * T, (2 * hf + 2) * T)
            cb = slice(M // 2 + 2 * hf * T, M // 2 + (2 * hf + 2) * T)
            for n, (r, c) in enumerate(((r1, ca), (r1, cb), (r2, ca), (r2, cb))):
                res = acc_ref[r, c] + jnp.concatenate([parts[0][n], parts[1][n]], axis=1)
                acc_ref[r, c] = res
                o_s[r, c] = res.astype(bf16)
            if hf == 1:
                @pl.when(s == NSTEP - 1)
                def _():
                    o_copy(b).start()

        order = list(range(NB - 1, -1, -1))
        projq(NP - 1, 0)
        projq(NP - 1, 1)
        qtodo = [(b, hf) for b in range(NP - 2, -1, -1) for hf in range(2)]
        otodo = []
        for i in order:
            ss = [scores(i, hh) for hh in range(HP)]
            fill = []
            if qtodo:
                fill.append(functools.partial(projq, *qtodo.pop(0)))
            if otodo:
                fill.append(functools.partial(outp, *otodo.pop(0)))
            for hh in range(HP):
                p, sc = softmax(i, ss[hh])
                if fill:
                    fill.pop(0)()
                ctx[(i, hh)] = pv(i, hh, p, sc)
            conv_inv(i)
            for fn in fill:
                fn()
            if i % 2 == 0:
                otodo += [(i // 2, 0), (i // 2, 1)]
        for a in otodo:
            outp(*a)
        assert not wwork

    kvo0 = kvo_copies(0)
    kvo0[0].start()
    kvo0[1].start()
    for cp in small:
        cp.start()
    c_copy.start()
    for cp in conv_copies(0):
        cp.start()
    q_copy(0).start()
    x_copies[0].start()
    kvo0[2].start()
    x_copies[1].start()

    def zero_body(i, carry):
        acc_ref[blk(i, T), :] = jnp.zeros((T, M), f32)
        return carry

    jax.lax.fori_loop(0, NB, zero_body, 0)
    bk_s[0:8, :] = jnp.zeros((8, T), u32)
    zm_s[...] = jnp.zeros((8, T), u32)
    kvo0[0].wait()
    kvo0[1].wait()
    for r0 in range(0, DC // 2, 16):
        wkv_piece(r0)
    kvo1 = kvo_copies(1)
    kvo1[0].start()
    kvo1[1].start()
    for cp in small:
        cp.wait()
    d_s[...] = dr_s[...].astype(f32)
    c_copy.wait()

    def comb_rows(src, dst, b, r0, nr, ncol):
        w1 = src[b * T + r0:b * T + r0 + nr, :]
        w2 = src[b * T + HF + r0:b * T + HF + r0 + nr, :]
        a1 = _upk(w1).astype(f32)
        a2 = _upk(w2).astype(f32)
        h = ncol // 2
        l7 = _lhs7(a1[:, :h], a1[:, h:], a2[:, :h], a2[:, h:])
        for j, jj in J5.items():
            rr = slice(jj * (S // 4) + b * HF + r0, jj * (S // 4) + b * HF + r0 + nr)
            dst[rr, :] = _pk(l7[j].astype(bf16))
        return a1, a2

    for b in range(NP):
        for r0 in range(0, HF, 8):
            comb_rows(c_s, c7_s, b, r0, 8, DC)

    def x_prep(b0, b1):
        gw = gw_s[...].astype(f32)
        for b in range(b0, b1):
            for r0 in range(0, HF, 8):
                rows = comb_rows(x_s, x7_s, b, r0, 8, M)
                for half, xf in enumerate(rows):
                    t = xf[:, 0:T] * gw[0:1, :]
                    for j in range(1, M // T):
                        t = t + xf[:, j * T:(j + 1) * T] * gw[j:j + 1, :]
                    z = jnp.sum(t, axis=-1, keepdims=True)
                    g = 0.5 * jnp.tanh(0.5 * z) + 0.5
                    g0 = b * 2 * T + half * T + 2 * r0
                    g_s[g0:g0 + 16, :] = jnp.broadcast_to(g, (16, T))

    def loop_body(s, carry):
        @pl.when(s >= 0)
        def _():
            phase_b(s)

        @pl.when(s + 1 < NSTEP)
        def _():
            phase_a(s + 1)

        @pl.when(s < 0)
        def _():
            kvo0[2].wait()
            for c0 in range(0, M // 2, T):
                for r0 in range(0, D, 16):
                    wo_piece(0, r0, c0)
            kvo1[2].start()
            x_copies[0].wait()
            x_prep(0, NP // 2)
            x_copies[1].wait()
            x_prep(NP // 2, NP)
        return carry

    jax.lax.fori_loop(-1, NSTEP, loop_body, 0)
    for b in range(NP):
        o_copy(b).wait()


@jax.jit
def pallas_gated_mix__compressed_kv_cla__ssm_conv_h3__prompt_kernel(
    A_x: jax.Array,
    A_c_kv: jax.Array,
    A_w_q: jax.Array,
    A_w_uk: jax.Array,
    A_w_uv: jax.Array,
    A_w_o: jax.Array,
    B_q: jax.Array,
    B_k: jax.Array,
    B_v: jax.Array,
    B_shift_k: jax.Array,
    B_ssm_k: jax.Array,
    B_ssm_D: jax.Array,
    gate_w: jax.Array,
):
    del B_q
    tab = jnp.asarray(_dft_tables().astype(bf16))
    out = pl.pallas_call(
        _kernel,
        in_specs=[pl.BlockSpec(memory_space=pl.ANY)] * 13,
        out_specs=pl.BlockSpec(memory_space=pl.ANY),
        out_shape=jax.ShapeDtypeStruct((S, M), bf16),
        scratch_shapes=[
            pltpu.VMEM((S, M), f32),
            pltpu.VMEM((S // 2, M), u32),
            pltpu.VMEM((S // 2, DC), u32),
            pltpu.VMEM((5 * S // 4, M // 2), u32),
            pltpu.VMEM((5 * S // 4, DC // 2), u32),
            pltpu.VMEM((M, D), u32),
            pltpu.VMEM((DC, D), u32),
            pltpu.VMEM((DC, D), u32),
            pltpu.VMEM((HP * D, M), bf16),
            pltpu.VMEM((S // 2 + 8, T), u32),
            pltpu.VMEM((S // 2, T), u32),
            pltpu.VMEM((T, S), bf16),
            pltpu.VMEM((KS, M), bf16),
            pltpu.VMEM((M // T, T), bf16),
            pltpu.VMEM((M // T, T), bf16),
            pltpu.VMEM((6, T, T), bf16),
            pltpu.VMEM((M // 4, 7 * T), u32),
            pltpu.VMEM((DC // 4, 14 * T), u32),
            pltpu.VMEM((2 * 4 * HF, 7 * T), u32),
            pltpu.VMEM((S // 2, HP * D), u32),
            pltpu.VMEM((S // 2, HP * D), u32),
            pltpu.VMEM((S, T), f32),
            pltpu.VMEM((M // T, T), f32),
            pltpu.VMEM((S, M), bf16),
            pltpu.VMEM((S, T), f32),
            pltpu.VMEM((S, T), bf16),
            pltpu.VMEM((8, T), u32),
            pltpu.SemaphoreType.DMA((4,)),
            pltpu.SemaphoreType.DMA((3,)),
            pltpu.SemaphoreType.DMA((3,)),
            pltpu.SemaphoreType.DMA((4,)),
            pltpu.SemaphoreType.DMA(()),
        ],
        compiler_params=pltpu.CompilerParams(
            vmem_limit_bytes=100 * 1024 * 1024,
            disable_bounds_checks=True,
        ),
    )(
        A_x.reshape(S, M), A_c_kv.reshape(S, DC), A_w_q, A_w_uk, A_w_uv, A_w_o.reshape(H * D, M),
        B_k.reshape(S, M), B_v.reshape(S, M), B_shift_k.T, B_ssm_k,
        B_ssm_D.reshape(M // T, T), gate_w.reshape(M // T, T), tab,
    )
    return out.reshape(1, S, M)
```
